```python
import os as _os
_os.environ.setdefault("JAX_PLATFORMS", "cpu")
import jax
import jax.numpy as jnp

def _softmax(x, axis=-1):
    return jax.nn.softmax(x, axis=axis)
def _gelu(x):
    return jax.nn.gelu(x, approximate=True)
def _silu(x):
    return jax.nn.silu(x)
def _sigmoid(x):
    return jax.nn.sigmoid(x)
def _layernorm(x, axis=-1, eps=1e-5):
    m = jnp.mean(x, axis=axis, keepdims=True)
    v = jnp.var(x, axis=axis, keepdims=True)
    return (x - m) / jnp.sqrt(v + eps)
def _scatter_add(tgt, idx, src, axis=0):
    return tgt.at[idx].add(src)
def _segment_sum(src, seg, n):
    return jax.ops.segment_sum(src, seg, n)
class _Rng:
    def __init__(self, key):
        self._k = key
    def _next(self):
        self._k, sub = jax.random.split(self._k)
        return sub
    def normal(self, shape):
        return jax.random.normal(self._next(), shape, dtype=jnp.bfloat16)
    def randint(self, lo, hi, shape):
        return jax.random.randint(self._next(), shape, lo, hi, dtype=jnp.int32)
    def uniform(self, shape, lo=0.0, hi=1.0):
        return jax.random.uniform(self._next(), shape, jnp.bfloat16, lo, hi)
    def permutation(self, n):
        return jax.random.permutation(self._next(), n)


kernel_name = 'gated_mix__gqa_block_cached__dense_activation_squared_relu__decode'

def setup_inputs():
    _rng = _Rng(jax.random.key(int.from_bytes(__import__("os").urandom(4), "little")))
    _w = (lambda a: (lambda t: t.astype(jnp.bfloat16) if jnp.issubdtype(t.dtype, jnp.floating) else t)(jnp.asarray(a)))
    def _A_setup():
        B, Sq, D = 4, 1, 512
        Hq, Hkv, Sk, Dh = 32, 8, 4096, 128
        assert Hq % Hkv == 0, (Hq, Hkv)
        return {
            "x": _w((lambda *s: _rng.normal(s) * 0.05)(B, Sq, D)),
            "k_cache": _w((lambda *s: _rng.normal(s) * 3.2)(B, Hkv, Sk, Dh)),
            "v_cache": _w((lambda *s: _rng.normal(s) * 1.6)(B, Hkv, Sk, Dh)),
            "wq": _w((lambda *s: _rng.normal(s) * 3.2)(D, Hq * Dh) * (D ** -0.5)),
            "wo": _w((lambda *s: _rng.normal(s) * 1.6)(Hq * Dh, D) * ((Hq * Dh) ** -0.5)),
        }
    _A_in = _A_setup()

    def _B_setup():
        B, S, D, F = 4, 1, 512, 1792
        return {
            "x": _w((lambda *s: _rng.normal(s) * 0.05)(B, S, D)),
            "w1": _w((lambda *s: _rng.normal(s) * 0.1)(D, F)),
            "b1": _w((lambda *s: _rng.normal(s) * 0.05)(F)),
            "w2": _w((lambda *s: _rng.normal(s) * 0.05)(F, D)),
            "b2": _w((lambda *s: _rng.normal(s) * 0.05)(D)),
        }
    _B_in = _B_setup()

    return {
        "A_x": _A_in["x"],
        "A_k_cache": _A_in["k_cache"],
        "A_v_cache": _A_in["v_cache"],
        "A_wq": _A_in["wq"],
        "A_wo": _A_in["wo"],
        "B_x": _B_in["x"],
        "B_w1": _B_in["w1"],
        "B_b1": _B_in["b1"],
        "B_w2": _B_in["w2"],
        "B_b2": _B_in["b2"],
        "gate_w": _w((lambda *s: _rng.normal(s) * 0.05)(512) * 16.0),
    }

def reference(A_x, A_k_cache, A_v_cache, A_wq, A_wo, B_x, B_w1, B_b1, B_w2, B_b2, gate_w):
    def _A_ref(x, k_cache, v_cache, wq, wo):
        B, Sq, D = x.shape
        Hq, Dh = 32, 128
        Hkv = k_cache.shape[1]
        rep = Hq // Hkv
        q = (lambda x, *d: x.transpose(*d))((x @ wq).reshape(B, Sq, Hq, Dh), 0, 2, 1, 3)
        k = jnp.repeat(k_cache, rep, axis=1)
        v = jnp.repeat(v_cache, rep, axis=1)
        scores = jnp.einsum("bhqd,bhkd->bhqk", q, k) * (Dh ** -0.5)
        p = _softmax(scores, axis=-1)
        o = jnp.einsum("bhqk,bhkd->bhqd", p, v)
        return (lambda x, *d: x.transpose(*d))(o, 0, 2, 1, 3).reshape(B, Sq, Hq * Dh) @ wo

    def _B_ref(x, w1, b1, w2, b2):
        h = jnp.einsum("bsd,df->bsf", x, w1) + b1
        zero = jnp.zeros_like(h)
        r = jnp.where(h > zero, h, zero)
        h = r * r
        out = jnp.einsum("bsf,fd->bsd", h, w2) + b2
        return out

    x = A_x
    g = _sigmoid((x * gate_w).sum(-1, keepdims=True))
    a = _A_ref(x, A_k_cache, A_v_cache, A_wq, A_wo)
    b = _B_ref(x, B_w1, B_b1, B_w2, B_b2)
    return g * a + (1 - g) * b
```

```python
import jax
import jax.numpy as jnp
from jax import lax
import jax.experimental.pallas as pl
import jax.experimental.pallas.tpu as pltpu

B, D, HQ, HKV, SK, DH, F = 4, 512, 32, 8, 4096, 128, 1792
REP = HQ // HKV
GW = REP * DH
SCALE = float(DH) ** -0.5
f32 = jnp.float32
bf16 = jnp.bfloat16


def _kernel(x_hbm, k_hbm, v_hbm, wq_hbm, wo_hbm, w1_hbm, b1_hbm, w2_hbm, b2_hbm, gw_hbm,
            o_ref,
            x_v, gw_v, b1_v, b2_v, w1_v, w2_v, wq_v, wo_v, kbuf, vbuf, q_scr, o_scr,
            sem_s, sem_w, sem_k, sem_v):
    def cp_small():
        return [
            pltpu.make_async_copy(x_hbm, x_v, sem_s.at[0]),
            pltpu.make_async_copy(gw_hbm, gw_v, sem_s.at[1]),
            pltpu.make_async_copy(b1_hbm, b1_v, sem_s.at[2]),
            pltpu.make_async_copy(b2_hbm, b2_v, sem_s.at[3]),
        ]

    def cp_wq(h):
        return pltpu.make_async_copy(
            wq_hbm.at[:, pl.ds(pl.multiple_of(h * GW, GW), GW)], wq_v, sem_w.at[0])

    def cp_wo(h):
        return pltpu.make_async_copy(
            wo_hbm.at[pl.ds(pl.multiple_of(h * GW, GW), GW), :], wo_v, sem_w.at[1])

    def cp_w1():
        return pltpu.make_async_copy(w1_hbm, w1_v, sem_w.at[2])

    def cp_w2():
        return pltpu.make_async_copy(w2_hbm, w2_v, sem_w.at[3])

    def cp_k(b, h):
        return pltpu.make_async_copy(k_hbm.at[b, h], kbuf.at[b], sem_k.at[b])

    def cp_v(b, h):
        return pltpu.make_async_copy(v_hbm.at[b, h], vbuf.at[b], sem_v.at[b])

    smalls = cp_small()
    smalls[0].start()
    cp_wq(0).start()
    cp_k(0, 0).start()
    cp_v(0, 0).start()
    for c in smalls[1:]:
        c.start()
    for b in range(1, B):
        cp_k(b, 0).start()
        cp_v(b, 0).start()
    cp_wo(0).start()
    cp_w1().start()
    cp_w2().start()

    q_scr[...] = jnp.zeros_like(q_scr)
    o_scr[...] = jnp.zeros_like(o_scr)
    smalls[0].wait()
    x = x_v[...]

    def head_step(h, acc):
        last = h + 1 >= HKV
        hn = jnp.minimum(h + 1, HKV - 1)
        cp_wq(h).wait()
        qh = jnp.dot(x, wq_v[...], preferred_element_type=f32)

        @pl.when(jnp.logical_not(last))
        def _():
            cp_wq(hn).start()

        for r in range(REP):
            q_scr[pl.ds(r, B, stride=8), :] = qh[:, r * DH:(r + 1) * DH]

        for b in range(B):
            qb = q_scr[b * 8:(b + 1) * 8, :].astype(bf16)
            cp_k(b, h).wait()
            s = lax.dot_general(qb, kbuf[b], (((1,), (1,)), ((), ())),
                                preferred_element_type=f32) * SCALE

            @pl.when(jnp.logical_not(last))
            def _():
                cp_k(b, hn).start()

            m = jnp.max(s, axis=-1, keepdims=True)
            p = jnp.exp(s - m)
            l = jnp.sum(p, axis=-1, keepdims=True)
            cp_v(b, h).wait()
            o = jnp.dot(p.astype(bf16), vbuf[b], preferred_element_type=f32)

            @pl.when(jnp.logical_not(last))
            def _():
                cp_v(b, hn).start()

            o = o / l
            o_scr[pl.ds(b, REP, stride=8), :] = o[0:REP, :]

        oh = jnp.concatenate([o_scr[r * 8:(r + 1) * 8, :] for r in range(REP)], axis=1)
        cp_wo(h).wait()
        acc = acc + jnp.dot(oh.astype(bf16), wo_v[...], preferred_element_type=f32)

        @pl.when(jnp.logical_not(last))
        def _():
            cp_wo(hn).start()

        return acc

    acc = lax.fori_loop(0, HKV, head_step, jnp.zeros((8, D), f32))

    for c in smalls[1:]:
        c.wait()
    cp_w1().wait()
    hh = jnp.dot(x, w1_v[...], preferred_element_type=f32) + b1_v[...].astype(f32)[None, :]
    r = jnp.maximum(hh, 0.0)
    r2 = (r * r).astype(bf16)
    cp_w2().wait()
    ffn = jnp.dot(r2, w2_v[...], preferred_element_type=f32) + b2_v[...].astype(f32)[None, :]
    gl = jnp.sum(x.astype(f32) * gw_v[...].astype(f32)[None, :], axis=-1, keepdims=True)
    g = jax.nn.sigmoid(gl)
    o_ref[...] = (g * acc[0:B, :] + (1.0 - g) * ffn).astype(o_ref.dtype)


@jax.jit
def pallas_gated_mix__gqa_block_cached__dense_activation_squared_relu__decode_kernel(
    A_x, A_k_cache, A_v_cache, A_wq, A_wo, B_x, B_w1, B_b1, B_w2, B_b2, gate_w,
):
    del B_x
    x = A_x.reshape(B, D)
    hbm = pl.BlockSpec(memory_space=pltpu.HBM)
    out = pl.pallas_call(
        _kernel,
        out_shape=jax.ShapeDtypeStruct((B, D), bf16),
        in_specs=[hbm] * 10,
        out_specs=pl.BlockSpec(memory_space=pltpu.VMEM),
        scratch_shapes=[
            pltpu.VMEM((B, D), bf16),
            pltpu.VMEM((D,), bf16),
            pltpu.VMEM((F,), bf16),
            pltpu.VMEM((D,), bf16),
            pltpu.VMEM((D, F), bf16),
            pltpu.VMEM((F, D), bf16),
            pltpu.VMEM((D, GW), bf16),
            pltpu.VMEM((GW, D), bf16),
            pltpu.VMEM((B, SK, DH), bf16),
            pltpu.VMEM((B, SK, DH), bf16),
            pltpu.VMEM((B * 8, DH), f32),
            pltpu.VMEM((REP * 8, DH), f32),
            pltpu.SemaphoreType.DMA((4,)),
            pltpu.SemaphoreType.DMA((4,)),
            pltpu.SemaphoreType.DMA((B,)),
            pltpu.SemaphoreType.DMA((B,)),
        ],
        compiler_params=pltpu.CompilerParams(vmem_limit_bytes=64 * 1024 * 1024),
    )(x, A_k_cache, A_v_cache, A_wq, A_wo, B_w1, B_b1, B_w2, B_b2, gate_w)
    return out.reshape(B, 1, D)
```

```python
import jax
import jax.numpy as jnp
from jax import lax
import jax.experimental.pallas as pl
import jax.experimental.pallas.tpu as pltpu

B, D, HQ, HKV, SK, DH, F = 4, 512, 32, 8, 4096, 128, 1792
REP = HQ // HKV
GW = REP * DH
SCALE = float(DH) ** -0.5
f32 = jnp.float32
bf16 = jnp.bfloat16
NKV = 2 * B
NQ = 4


def build(dist=4, ck=16, run=8, unroll=2, nobc=False, pure=False, wo_split=(1024, 1024, 1024, 512, 512), ck_w1=16, run_w1=2,
          ck_w2=16, run_w2=8, full_unroll=False, nosc=False):
    assert dist <= NKV
    wo_edges = [0]
    for r_ in wo_split:
        wo_edges.append(wo_edges[-1] + r_)
    assert wo_edges[-1] == HQ * DH
    NC = 2 + len(wo_split)
    NS = NKV if NKV % dist else dist
    assert NKV % NS == 0 and NS >= dist

    def _kernel(x_hbm, k_hbm, v_hbm, wq_hbm, wo_hbm, w1_hbm, b1_hbm, w2_hbm, b2_hbm, gw_hbm,
                o_ref,
                x_v, gw_v, b1_v, b2_v, wq_v, w1_v, w2_v, wo_v, kbuf, vbuf, q_scr, o_scr, mix_scr, g_scr,
                sem_s, sem_r):

        def start_rows(src, dst, sem, rows, run):
            n = dst.shape[0] // rows
            run = max(1, min(run, n // 2))
            assert n * rows == dst.shape[0] and n % (2 * run) == 0, (dst.shape, rows, run)

            def body(blk, c):
                base = pl.multiple_of(blk * (2 * run * rows), 2 * run * rows)
                for r in range(run):
                    for p in range(2):
                        sl = pl.ds(base + (p * run + r) * rows, rows)
                        pltpu.make_async_copy(src.at[sl], dst.at[sl], sem).start(priority=p)
                return c
            nblk = n // (2 * run)
            if nblk == 1:
                body(0, 0)
            else:
                lax.fori_loop(0, nblk, body, 0, unroll=(nblk if full_unroll else 1))

        def start_wq(c):
            cw = ck * 1024 // 32
            ncol = (HQ * DH) // cw
            reg = ck * run
            if reg >= 128:
                gpr = reg // 128
                def body(blk, carry):
                    r0 = pl.multiple_of(c * 128 + blk * (2 * gpr * 16), 16)
                    for r in range(gpr * ncol):
                        for p in range(2):
                            rs = pl.ds(r0 + (p * gpr + r // ncol) * 16, 16)
                            cs = pl.ds((r % ncol) * cw, cw)
                            pltpu.make_async_copy(wq_hbm.at[rs, cs], wq_v.at[rs, cs], sem_r.at[c % NS]).start(priority=p)
                    return carry
                lax.fori_loop(0, 8 // (2 * gpr), body, 0)
            else:
                def body(i, carry):
                    half = ncol // 2
                    rg, r = i // half, i % half
                    blk, rr = r // run, r % run
                    for p in range(2):
                        rs = pl.ds(pl.multiple_of(c * 128 + rg * 16, 16), 16)
                        cs = pl.ds(pl.multiple_of(((2 * blk + p) * run + rr) * cw, cw), cw)
                        pltpu.make_async_copy(wq_hbm.at[rs, cs], wq_v.at[rs, cs], sem_r.at[c % NS]).start(priority=p)
                    return carry
                lax.fori_loop(0, 8 * ncol // 2, body, 0, unroll=unroll)

        def wait_all(dst, sem):
            pltpu.make_async_copy(dst, dst, sem).wait()

        def kv_item(j, h):
            b, isv = j // 2, j % 2
            if isv:
                return v_hbm.at[b, h], vbuf.at[b], sem_r.at[(NQ + j) % NS]
            return k_hbm.at[b, h], kbuf.at[b], sem_r.at[(NQ + j) % NS]

        def start_kv(j, h):
            src, dst, sem = kv_item(j, h)
            start_rows(src, dst, sem, ck * 4, run)

        def wait_kv(j, h):
            _, dst, sem = kv_item(j, h)
            wait_all(dst, sem)
            return dst

        def c_item(i):
            if i == 0:
                return w1_hbm, w1_v, sem_r.at[(NQ + NKV * HKV + i) % NS], ck_w1, run_w1
            if i == 1:
                return w2_hbm, w2_v, sem_r.at[(NQ + NKV * HKV + i) % NS], ck_w2, run_w2
            lo, hi = wo_edges[i - 2], wo_edges[i - 1]
            return wo_hbm.at[lo:hi], wo_v.at[lo:hi], sem_r.at[(NQ + NKV * HKV + i) % NS], ck, run

        def start_c(i):
            if i < NC:
                src, dst, sem, rows, rn = c_item(i)
                start_rows(src, dst, sem, rows, rn)

        def wait_c(i):
            _, dst, sem, _, _ = c_item(i)
            wait_all(dst, sem)

        def refill(j, h):
            jn = j + dist
            if jn < NKV:
                start_kv(jn, h)
            else:
                @pl.when(h + 1 < HKV)
                def _():
                    start_kv(jn - NKV, jnp.minimum(h + 1, HKV - 1))

                @pl.when(h + 1 == HKV)
                def _():
                    start_c(jn - NKV)

        smalls = [
            pltpu.make_async_copy(x_hbm, x_v, sem_s),
            pltpu.make_async_copy(gw_hbm, gw_v, sem_s),
            pltpu.make_async_copy(b1_hbm, b1_v, sem_s),
            pltpu.make_async_copy(b2_hbm, b2_v, sem_s),
        ]
        start_wq(0)
        for c in smalls:
            c.start()
        for c in range(1, min(dist, NQ)):
            start_wq(c)
        for j in range(max(0, dist - NQ)):
            start_kv(j, 0)

        def after_wq(c):
            i = c + dist
            if i < NQ:
                start_wq(i)
            else:
                start_kv(i - NQ, 0)

        if pure:
            for c in smalls:
                c.wait()
            for c in range(NQ):
                wait_all(wq_v.at[c * 128:(c + 1) * 128], sem_r.at[c % NS])
                after_wq(c)

            def pstep(h, c):
                for j in range(NKV):
                    wait_kv(j, h)
                    refill(j, h)
                return c
            lax.fori_loop(0, HKV, pstep, 0)
            for i in range(NC):
                wait_c(i)
                start_c(i + dist)
            o_ref[...] = jnp.zeros_like(o_ref)
            return

        q_scr[...] = jnp.zeros_like(q_scr)
        o_scr[...] = jnp.zeros_like(o_scr)
        for c in smalls:
            c.wait()
        x = x_v[...]

        q = None
        for c in range(NQ):
            wait_all(wq_v.at[c * 128:(c + 1) * 128], sem_r.at[c % NS])
            part = jnp.dot(x[:, c * 128:(c + 1) * 128], wq_v[c * 128:(c + 1) * 128, :], preferred_element_type=f32)
            q = part if q is None else q + part
            after_wq(c)
        for hq in range(HQ):
            q_scr[hq // REP, pl.ds(hq % REP, B, stride=8), :] = q[:, hq * DH:(hq + 1) * DH]

        def head_step(h, carry):
            for b in range(B):
                qb = q_scr[h, b * 8:(b + 1) * 8, :].astype(bf16)
                k_ref = wait_kv(2 * b, h)
                s = lax.dot_general(qb, k_ref[...], (((1,), (1,)), ((), ())),
                                    preferred_element_type=f32) * SCALE
                refill(2 * b, h)
                m = jnp.max(s, axis=-1, keepdims=True)
                p = jnp.exp(s - m)
                l = jnp.sum(p, axis=-1, keepdims=True)
                v_ref = wait_kv(2 * b + 1, h)
                o = jnp.dot(p.astype(bf16), v_ref[...], preferred_element_type=f32)
                refill(2 * b + 1, h)
                o = o / l
                o_scr[h, pl.ds(b, REP, stride=8), :] = o[0:REP, :]
            return carry

        lax.fori_loop(0, HKV, head_step, 0)

        wait_c(0)
        hh = jnp.dot(x, w1_v[...], preferred_element_type=f32) + b1_v[...].astype(f32)[None, :]
        start_c(0 + dist)
        r = jnp.maximum(hh, 0.0)
        r2 = (r * r).astype(bf16)
        wait_c(1)
        ffn = jnp.dot(r2, w2_v[...], preferred_element_type=f32) + b2_v[...].astype(f32)[None, :]
        start_c(1 + dist)
        gl = jnp.sum(x.astype(f32) * gw_v[...].astype(f32)[None, :], axis=-1, keepdims=True)
        g = jax.nn.sigmoid(gl)
        mix = (1.0 - g) * ffn
        acc = None
        for i in range(2, NC):
            lo, hi = wo_edges[i - 2], wo_edges[i - 1]
            parts = []
            for hq in range(lo // DH, hi // DH):
                h_, r_ = hq // REP, hq % REP
                parts.append(o_scr[h_, r_ * 8:(r_ + 1) * 8, :])
            oh = jnp.concatenate(parts, axis=1).astype(bf16)
            wait_c(i)
            part = jnp.dot(oh, wo_v[lo:hi, :], preferred_element_type=f32)
            acc = part if acc is None else acc + part
            start_c(i + dist)
        o_ref[...] = (g * acc[0:B, :] + mix).astype(o_ref.dtype)

    def fn(A_x, A_k_cache, A_v_cache, A_wq, A_wo, B_x, B_w1, B_b1, B_w2, B_b2, gate_w):
        del B_x
        x = A_x.reshape(B, D)
        hbm = pl.BlockSpec(memory_space=pltpu.HBM)
        out = pl.pallas_call(
            _kernel,
            out_shape=jax.ShapeDtypeStruct((B, D), bf16),
            in_specs=[hbm] * 10,
            out_specs=pl.BlockSpec(memory_space=pltpu.VMEM),
            scratch_shapes=[
                pltpu.VMEM((B, D), bf16), pltpu.VMEM((D,), bf16), pltpu.VMEM((F,), bf16), pltpu.VMEM((D,), bf16),
                pltpu.VMEM((D, HQ * DH), bf16), pltpu.VMEM((D, F), bf16), pltpu.VMEM((F, D), bf16),
                pltpu.VMEM((HQ * DH, D), bf16),
                pltpu.VMEM((B, SK, DH), bf16), pltpu.VMEM((B, SK, DH), bf16),
                pltpu.VMEM((HKV, B * 8, DH), f32), pltpu.VMEM((HKV, REP * 8, DH), f32),
                pltpu.VMEM((B, D), f32), pltpu.VMEM((B, DH), f32),
                pltpu.SemaphoreType.DMA(()), pltpu.SemaphoreType.DMA((NS,)),
            ],
            compiler_params=pltpu.CompilerParams(vmem_limit_bytes=64 * 1024 * 1024, disable_bounds_checks=nobc, disable_semaphore_checks=nosc),
        )(x, A_k_cache, A_v_cache, A_wq, A_wo, B_w1, B_b1, B_w2, B_b2, gate_w)
        return out.reshape(B, 1, D)

    return fn


_fn = build(run=16, wo_split=(1024, 1024, 1024, 512, 256, 256))


@jax.jit
def pallas_gated_mix__gqa_block_cached__dense_activation_squared_relu__decode_kernel(
    A_x, A_k_cache, A_v_cache, A_wq, A_wo, B_x, B_w1, B_b1, B_w2, B_b2, gate_w,
):
    return _fn(A_x, A_k_cache, A_v_cache, A_wq, A_wo, B_x, B_w1, B_b1, B_w2, B_b2, gate_w)
```

```python
import jax
import jax.numpy as jnp
from jax import lax
import jax.experimental.pallas as pl
import jax.experimental.pallas.tpu as pltpu

B, D, HQ, HKV, SK, DH, F = 4, 512, 32, 8, 4096, 128, 1792
REP = HQ // HKV
QW = HQ * DH
SCALE = float(DH) ** -0.5

CHUNK_ROWS = 16
KV_ROWS = 64
WO_TAIL = 256

f32 = jnp.float32
bf16 = jnp.bfloat16


def _kernel(x_hbm, k_hbm, v_hbm, wq_hbm, wo_hbm, w1_hbm, b1_hbm, w2_hbm, b2_hbm, gw_hbm,
            o_ref,
            x_v, gw_v, b1_v, b2_v, wq_v, w1_v, w2_v, wo_v, kbuf, vbuf,
            q_scr, o_scr, mix_scr, g_scr, sem_ring, sem_tail):

    def start_pair(src0, dst0, sem0, rows0, src1, dst1, sem1, rows1, per0=1, per1=1, unroll=8):
        steps = dst0.shape[0] // (rows0 * per0)
        assert steps * rows0 * per0 == dst0.shape[0] and steps * rows1 * per1 == dst1.shape[0]
        unroll = min(unroll, steps)
        assert steps % unroll == 0

        def body(i, carry):
            for t in range(unroll):
                for a in range(per0):
                    sl = pl.ds(pl.multiple_of(((i * unroll + t) * per0 + a) * rows0, rows0), rows0)
                    pltpu.make_async_copy(src0.at[sl], dst0.at[sl], sem0).start(priority=0)
                for a in range(per1):
                    sl = pl.ds(pl.multiple_of(((i * unroll + t) * per1 + a) * rows1, rows1), rows1)
                    pltpu.make_async_copy(src1.at[sl], dst1.at[sl], sem1).start(priority=1)
            return carry

        if steps == unroll:
            body(0, 0)
        else:
            lax.fori_loop(0, steps // unroll, body, 0)

    def wait_all(dst, sem):
        pltpu.make_async_copy(dst, dst, sem).wait()

    def sems(i):
        return sem_ring.at[2 * (i % 2)], sem_ring.at[2 * (i % 2) + 1]

    def start_wq():
        s0, s1 = sems(0)
        ncol = QW // D

        def body(rg, carry):
            r0 = pl.multiple_of(rg * CHUNK_ROWS, CHUNK_ROWS)
            for c in range(ncol):
                cs = pl.ds(c * D, D)
                for prio, sem in ((0, s0), (1, s1)):
                    rs = pl.ds(r0 + prio * (D // 2), CHUNK_ROWS)
                    pltpu.make_async_copy(wq_hbm.at[rs, cs], wq_v.at[rs, cs], sem).start(priority=prio)
            return carry

        lax.fori_loop(0, D // 2 // CHUNK_ROWS, body, 0)

    def start_ffn_weights():
        s0, s1 = sems(1)
        start_pair(w1_hbm, w1_v, s0, CHUNK_ROWS, w2_hbm, w2_v, s1, CHUNK_ROWS, per0=2, per1=7)

    def start_kv(b, h):
        s0, s1 = sems(b)
        start_pair(k_hbm.at[b, h], kbuf.at[b], s0, KV_ROWS, v_hbm.at[b, h], vbuf.at[b], s1, KV_ROWS)

    def start_wo_rows(lo0, lo1, n, sem0, sem1):
        start_pair(wo_hbm.at[lo0:lo0 + n], wo_v.at[lo0:lo0 + n], sem0, CHUNK_ROWS,
                   wo_hbm.at[lo1:lo1 + n], wo_v.at[lo1:lo1 + n], sem1, CHUNK_ROWS)

    def start_wo(slab):
        s0, s1 = sems(slab)
        half, n = QW // 2, QW // 4
        if slab == 0:
            start_wo_rows(0, half, n, s0, s1)
        else:
            start_wo_rows(n, half + n, n - WO_TAIL, s0, s1)
            start_wo_rows(2 * n - WO_TAIL, QW - WO_TAIL, WO_TAIL, s0, sem_tail)

    def refill(b, h):
        if b + 2 < B:
            start_kv(b + 2, h)
        else:
            @pl.when(h + 1 < HKV)
            def _():
                start_kv(b + 2 - B, jnp.minimum(h + 1, HKV - 1))

            @pl.when(h + 1 == HKV)
            def _():
                start_wo(b + 2 - B)

    smalls = [pltpu.make_async_copy(src, dst, sems(0)[0])
              for src, dst in ((x_hbm, x_v), (gw_hbm, gw_v), (b1_hbm, b1_v), (b2_hbm, b2_v))]

    start_wq()
    for c in smalls:
        c.start()
    start_ffn_weights()
    q_scr[...] = jnp.zeros_like(q_scr)
    o_scr[...] = jnp.zeros_like(o_scr)

    s0, s1 = sems(0)
    wait_all(wq_v.at[0:D // 2], s0)
    wait_all(wq_v.at[D // 2:D], s1)
    for c in smalls:
        c.wait()
    x = x_v[...]
    q = jnp.dot(x, wq_v[...], preferred_element_type=f32)
    start_kv(0, 0)
    for hq in range(HQ):
        q_scr[hq // REP, pl.ds(hq % REP, B, stride=8), :] = q[:, hq * DH:(hq + 1) * DH]

    s0, s1 = sems(1)
    wait_all(w1_v, s0)
    hid = jnp.dot(x, w1_v[...], preferred_element_type=f32) + b1_v[...].astype(f32)[None, :]
    hid = jnp.where(hid > 0.0, hid, 0.0)
    hid = (hid * hid).astype(bf16)
    wait_all(w2_v, s1)
    ffn = jnp.dot(hid, w2_v[...], preferred_element_type=f32) + b2_v[...].astype(f32)[None, :]
    g = jax.nn.sigmoid(jnp.sum(x.astype(f32) * gw_v[...].astype(f32)[None, :], axis=-1, keepdims=True))
    mix_scr[...] = (1.0 - g) * ffn
    g_scr[...] = jnp.broadcast_to(g, (B, DH))
    start_kv(1, 0)

    def head_step(h, carry):
        for b in range(B):
            s0, s1 = sems(b)
            qb = q_scr[h, b * 8:(b + 1) * 8, :].astype(bf16)
            wait_all(kbuf.at[b], s0)
            s = lax.dot_general(qb, kbuf[b], (((1,), (1,)), ((), ())),
                                preferred_element_type=f32) * SCALE
            m = jnp.max(s, axis=-1, keepdims=True)
            p = jnp.exp(s - m)
            l = jnp.sum(p, axis=-1, keepdims=True)
            wait_all(vbuf.at[b], s1)
            o = jnp.dot(p.astype(bf16), vbuf[b], preferred_element_type=f32)
            refill(b, h)
            o = o / l
            o_scr[h, pl.ds(b, REP, stride=8), :] = o[0:REP, :]
        return carry

    lax.fori_loop(0, HKV, head_step, 0)

    (a0, a1), (b0, b1) = sems(0), sems(1)
    half, n = QW // 2, QW // 4
    pieces = [(0, n, a0), (half, half + n, a1), (n, half, b0),
              (half + n, QW - WO_TAIL, b1), (QW - WO_TAIL, QW, sem_tail)]
    acc = None
    for lo, hi, sem in pieces:
        heads = [o_scr[hq // REP, (hq % REP) * 8:(hq % REP + 1) * 8, :] for hq in range(lo // DH, hi // DH)]
        oh = jnp.concatenate(heads, axis=1).astype(bf16)
        wait_all(wo_v.at[lo:hi], sem)
        part = jnp.dot(oh, wo_v[lo:hi, :], preferred_element_type=f32)
        acc = part if acc is None else acc + part
    o_ref[...] = (g_scr[:, 0:1] * acc[0:B, :] + mix_scr[...]).astype(o_ref.dtype)


@jax.jit
def pallas_gated_mix__gqa_block_cached__dense_activation_squared_relu__decode_kernel(
    A_x: jax.Array,
    A_k_cache: jax.Array,
    A_v_cache: jax.Array,
    A_wq: jax.Array,
    A_wo: jax.Array,
    B_x: jax.Array,
    B_w1: jax.Array,
    B_b1: jax.Array,
    B_w2: jax.Array,
    B_b2: jax.Array,
    gate_w: jax.Array,
):
    del B_x
    hbm = pl.BlockSpec(memory_space=pltpu.HBM)
    out = pl.pallas_call(
        _kernel,
        out_shape=jax.ShapeDtypeStruct((B, D), A_x.dtype),
        in_specs=[hbm] * 10,
        out_specs=pl.BlockSpec(memory_space=pltpu.VMEM),
        scratch_shapes=[
            pltpu.VMEM((B, D), bf16),
            pltpu.VMEM((D,), bf16),
            pltpu.VMEM((F,), bf16),
            pltpu.VMEM((D,), bf16),
            pltpu.VMEM((D, QW), bf16),
            pltpu.VMEM((D, F), bf16),
            pltpu.VMEM((F, D), bf16),
            pltpu.VMEM((QW, D), bf16),
            pltpu.VMEM((B, SK, DH), bf16),
            pltpu.VMEM((B, SK, DH), bf16),
            pltpu.VMEM((HKV, B * 8, DH), f32),
            pltpu.VMEM((HKV, REP * 8, DH), f32),
            pltpu.VMEM((B, D), f32),
            pltpu.VMEM((B, DH), f32),
            pltpu.SemaphoreType.DMA((4,)),
            pltpu.SemaphoreType.DMA(()),
        ],
        compiler_params=pltpu.CompilerParams(vmem_limit_bytes=48 * 1024 * 1024),
    )(A_x.reshape(B, D), A_k_cache, A_v_cache, A_wq, A_wo, B_w1, B_b1, B_w2, B_b2, gate_w)
    return out.reshape(B, 1, D)
```

```python
import jax
import jax.numpy as jnp
from jax import lax
import jax.experimental.pallas as pl
import jax.experimental.pallas.tpu as pltpu

B, D, HQ, HKV, SK, DH, F = 4, 512, 32, 8, 4096, 128, 1792
REP = HQ // HKV
QW = HQ * DH
SCALE = float(DH) ** -0.5

CHUNK_ROWS = 16
KV_ROWS = 128
WO_TAIL = 256

f32 = jnp.float32
bf16 = jnp.bfloat16


def _kernel(x_hbm, k_hbm, v_hbm, wq_hbm, wo_hbm, w1_hbm, b1_hbm, w2_hbm, b2_hbm, gw_hbm,
            o_ref,
            x_v, gw_v, b1_v, b2_v, wq_v, w1_v, w2_v, wo_v, kbuf, vbuf,
            q_scr, o_scr, mix_scr, g_scr, sem_ring, sem_tail):

    def start_pair(src0, dst0, sem0, rows0, src1, dst1, sem1, rows1, per0=1, per1=1, unroll=8):
        steps = dst0.shape[0] // (rows0 * per0)
        assert steps * rows0 * per0 == dst0.shape[0] and steps * rows1 * per1 == dst1.shape[0]
        unroll = min(unroll, steps)
        assert steps % unroll == 0

        def body(i, carry):
            for t in range(unroll):
                for a in range(per0):
                    sl = pl.ds(pl.multiple_of(((i * unroll + t) * per0 + a) * rows0, rows0), rows0)
                    pltpu.make_async_copy(src0.at[sl], dst0.at[sl], sem0).start(priority=0)
                for a in range(per1):
                    sl = pl.ds(pl.multiple_of(((i * unroll + t) * per1 + a) * rows1, rows1), rows1)
                    pltpu.make_async_copy(src1.at[sl], dst1.at[sl], sem1).start(priority=1)
            return carry

        if steps == unroll:
            body(0, 0)
        else:
            lax.fori_loop(0, steps // unroll, body, 0)

    def wait_all(dst, sem):
        pltpu.make_async_copy(dst, dst, sem).wait()

    def sems(i):
        return sem_ring.at[2 * (i % 2)], sem_ring.at[2 * (i % 2) + 1]

    def start_wq():
        s0, s1 = sems(0)
        ncol = QW // D

        def body(rg, carry):
            r0 = pl.multiple_of(rg * CHUNK_ROWS, CHUNK_ROWS)
            for c in range(ncol):
                cs = pl.ds(c * D, D)
                for prio, sem in ((0, s0), (1, s1)):
                    rs = pl.ds(r0 + prio * (D // 2), CHUNK_ROWS)
                    pltpu.make_async_copy(wq_hbm.at[rs, cs], wq_v.at[rs, cs], sem).start(priority=prio)
            return carry

        lax.fori_loop(0, D // 2 // CHUNK_ROWS, body, 0)

    def start_ffn_weights():
        s0, s1 = sems(1)
        start_pair(w1_hbm, w1_v, s0, CHUNK_ROWS, w2_hbm, w2_v, s1, CHUNK_ROWS, per0=2, per1=7)

    def start_kv(t, h):
        s0, s1 = sems(t)
        unroll = 4

        def body(i, carry):
            for u in range(unroll):
                sl = pl.ds(pl.multiple_of((i * unroll + u) * KV_ROWS, KV_ROWS), KV_ROWS)
                for b in (2 * t, 2 * t + 1):
                    pltpu.make_async_copy(k_hbm.at[b, h, sl], kbuf.at[b, sl], s0).start(priority=0)
                    pltpu.make_async_copy(v_hbm.at[b, h, sl], vbuf.at[b, sl], s1).start(priority=1)
            return carry

        lax.fori_loop(0, SK // KV_ROWS // unroll, body, 0)

    def start_wo_rows(lo0, lo1, n, sem0, sem1):
        start_pair(wo_hbm.at[lo0:lo0 + n], wo_v.at[lo0:lo0 + n], sem0, CHUNK_ROWS,
                   wo_hbm.at[lo1:lo1 + n], wo_v.at[lo1:lo1 + n], sem1, CHUNK_ROWS)

    def start_wo(slab):
        s0, s1 = sems(slab)
        half, n = QW // 2, QW // 4
        if slab == 0:
            start_wo_rows(0, half, n, s0, s1)
        else:
            start_wo_rows(n, half + n, n - WO_TAIL, s0, s1)
            start_wo_rows(2 * n - WO_TAIL, QW - WO_TAIL, WO_TAIL, s0, sem_tail)

    def refill(t, h):
        @pl.when(h + 1 < HKV)
        def _():
            start_kv(t, jnp.minimum(h + 1, HKV - 1))

        @pl.when(h + 1 == HKV)
        def _():
            start_wo(t)

    smalls = [pltpu.make_async_copy(src, dst, sems(0)[0])
              for src, dst in ((x_hbm, x_v), (gw_hbm, gw_v), (b1_hbm, b1_v), (b2_hbm, b2_v))]

    start_wq()
    for c in smalls:
        c.start()
    start_ffn_weights()
    q_scr[...] = jnp.zeros_like(q_scr)
    o_scr[...] = jnp.zeros_like(o_scr)

    s0, s1 = sems(0)
    wait_all(wq_v.at[0:D // 2], s0)
    wait_all(wq_v.at[D // 2:D], s1)
    for c in smalls:
        c.wait()
    x = x_v[...]
    q = jnp.dot(x, wq_v[...], preferred_element_type=f32)
    start_kv(0, 0)
    for hq in range(HQ):
        q_scr[hq // REP, pl.ds(hq % REP, B, stride=8), :] = q[:, hq * DH:(hq + 1) * DH]

    s0, s1 = sems(1)
    wait_all(w1_v, s0)
    hid = jnp.dot(x, w1_v[...], preferred_element_type=f32) + b1_v[...].astype(f32)[None, :]
    hid = jnp.where(hid > 0.0, hid, 0.0)
    hid = (hid * hid).astype(bf16)
    wait_all(w2_v, s1)
    ffn = jnp.dot(hid, w2_v[...], preferred_element_type=f32) + b2_v[...].astype(f32)[None, :]
    g = jax.nn.sigmoid(jnp.sum(x.astype(f32) * gw_v[...].astype(f32)[None, :], axis=-1, keepdims=True))
    mix_scr[...] = (1.0 - g) * ffn
    g_scr[...] = jnp.broadcast_to(g, (B, DH))
    start_kv(1, 0)

    def head_step(h, carry):
        for t in range(B // 2):
            s0, s1 = sems(t)
            wait_all(kbuf.at[2 * t:2 * t + 2], s0)
            wait_all(vbuf.at[2 * t:2 * t + 2], s1)
            outs = []
            for b in (2 * t, 2 * t + 1):
                qb = q_scr[h, b * 8:(b + 1) * 8, :].astype(bf16)
                s = lax.dot_general(qb, kbuf[b], (((1,), (1,)), ((), ())),
                                    preferred_element_type=f32) * SCALE
                m = jnp.max(s, axis=-1, keepdims=True)
                p = jnp.exp(s - m)
                l = jnp.sum(p, axis=-1, keepdims=True)
                o = jnp.dot(p.astype(bf16), vbuf[b], preferred_element_type=f32)
                outs.append((b, o, l))
            refill(t, h)
            for b, o, l in outs:
                o_scr[h, pl.ds(b, REP, stride=8), :] = (o / l)[0:REP, :]
        return carry

    lax.fori_loop(0, HKV, head_step, 0)

    (a0, a1), (b0, b1) = sems(0), sems(1)
    half, n = QW // 2, QW // 4
    pieces = [(0, n, a0), (half, half + n, a1), (n, half, b0),
              (half + n, QW - WO_TAIL, b1), (QW - WO_TAIL, QW, sem_tail)]
    acc = None
    for lo, hi, sem in pieces:
        heads = [o_scr[hq // REP, (hq % REP) * 8:(hq % REP + 1) * 8, :] for hq in range(lo // DH, hi // DH)]
        oh = jnp.concatenate(heads, axis=1).astype(bf16)
        wait_all(wo_v.at[lo:hi], sem)
        part = jnp.dot(oh, wo_v[lo:hi, :], preferred_element_type=f32)
        acc = part if acc is None else acc + part
    o_ref[...] = (g_scr[:, 0:1] * acc[0:B, :] + mix_scr[...]).astype(o_ref.dtype)


@jax.jit
def pallas_gated_mix__gqa_block_cached__dense_activation_squared_relu__decode_kernel(
    A_x: jax.Array,
    A_k_cache: jax.Array,
    A_v_cache: jax.Array,
    A_wq: jax.Array,
    A_wo: jax.Array,
    B_x: jax.Array,
    B_w1: jax.Array,
    B_b1: jax.Array,
    B_w2: jax.Array,
    B_b2: jax.Array,
    gate_w: jax.Array,
):
    del B_x
    hbm = pl.BlockSpec(memory_space=pltpu.HBM)
    out = pl.pallas_call(
        _kernel,
        out_shape=jax.ShapeDtypeStruct((B, D), A_x.dtype),
        in_specs=[hbm] * 10,
        out_specs=pl.BlockSpec(memory_space=pltpu.VMEM),
        scratch_shapes=[
            pltpu.VMEM((B, D), bf16),
            pltpu.VMEM((D,), bf16),
            pltpu.VMEM((F,), bf16),
            pltpu.VMEM((D,), bf16),
            pltpu.VMEM((D, QW), bf16),
            pltpu.VMEM((D, F), bf16),
            pltpu.VMEM((F, D), bf16),
            pltpu.VMEM((QW, D), bf16),
            pltpu.VMEM((B, SK, DH), bf16),
            pltpu.VMEM((B, SK, DH), bf16),
            pltpu.VMEM((HKV, B * 8, DH), f32),
            pltpu.VMEM((HKV, REP * 8, DH), f32),
            pltpu.VMEM((B, D), f32),
            pltpu.VMEM((B, DH), f32),
            pltpu.SemaphoreType.DMA((4,)),
            pltpu.SemaphoreType.DMA(()),
        ],
        compiler_params=pltpu.CompilerParams(vmem_limit_bytes=48 * 1024 * 1024),
    )(A_x.reshape(B, D), A_k_cache, A_v_cache, A_wq, A_wo, B_w1, B_b1, B_w2, B_b2, gate_w)
    return out.reshape(B, 1, D)
```

```python
import jax
import jax.numpy as jnp
from jax import lax
import jax.experimental.pallas as pl
import jax.experimental.pallas.tpu as pltpu

B, D, HQ, HKV, SK, DH, F = 4, 512, 32, 8, 4096, 128, 1792
REP = HQ // HKV
QW = HQ * DH
SCALE = float(DH) ** -0.5

CHUNK_ROWS = 16
KV_ROWS = 128
WO_TAIL = 256
SLOT_BATCH = (0, 2, 1, 3)

f32 = jnp.float32
bf16 = jnp.bfloat16


def _kernel(x_hbm, k_hbm, v_hbm, wq_hbm, wo_hbm, w1_hbm, b1_hbm, w2_hbm, b2_hbm, gw_hbm,
            o_ref,
            x_v, gw_v, b1_v, b2_v, wq_v, w1_v, w2_v, wo_v, kbuf, vbuf,
            q_scr, o_scr, mix_scr, g_scr, sem_ring, sem_tail):

    def wait_all(dst, sem):
        pltpu.make_async_copy(dst, dst, sem).wait()

    def sems(i):
        return sem_ring.at[2 * (i % 2)], sem_ring.at[2 * (i % 2) + 1]

    def start_wq():
        s0, s1 = sems(0)

        def body(rg, carry):
            r0 = pl.multiple_of(rg * CHUNK_ROWS, CHUNK_ROWS)
            for c in range(QW // 1024):
                cs = pl.ds(c * 1024, 1024)
                for w in range(2):
                    for prio, sem in ((0, s0), (1, s1)):
                        rs = pl.ds(r0 + prio * (D // 2) + w * (D // 4), CHUNK_ROWS)
                        pltpu.make_async_copy(wq_hbm.at[rs, cs], wq_v.at[rs, cs], sem).start(priority=prio)
            return carry

        lax.fori_loop(0, D // 4 // CHUNK_ROWS, body, 0)

    def start_ffn_weights():
        s0, s1 = sems(1)

        def body(i, carry):
            for a in range(7):
                for w in range(2):
                    if a < 4:
                        sl = pl.ds(pl.multiple_of(w * (D // 2) + (i * 4 + a) * 16, 16), 16)
                        pltpu.make_async_copy(w1_hbm.at[sl], w1_v.at[sl], s0).start(priority=0)
                    sl = pl.ds(pl.multiple_of(w * (F // 2) + (i * 7 + a) * 32, 32), 32)
                    pltpu.make_async_copy(w2_hbm.at[sl], w2_v.at[sl], s1).start(priority=1)
            return carry

        lax.fori_loop(0, 4, body, 0)

    def start_kv(t, h):
        s0, s1 = sems(t)
        unroll = 4

        def body(i, carry):
            for u in range(unroll):
                sl = pl.ds(pl.multiple_of((i * unroll + u) * KV_ROWS, KV_ROWS), KV_ROWS)
                for slot in (2 * t, 2 * t + 1):
                    b = SLOT_BATCH[slot]
                    pltpu.make_async_copy(k_hbm.at[b, h, sl], kbuf.at[slot, sl], s0).start(priority=0)
                    pltpu.make_async_copy(v_hbm.at[b, h, sl], vbuf.at[slot, sl], s1).start(priority=1)
            return carry

        lax.fori_loop(0, SK // KV_ROWS // unroll, body, 0)

    def start_wo_rows(lo0, lo1, n, sem0, sem1):
        unroll = 8
        assert n % (unroll * CHUNK_ROWS) == 0

        def body(i, carry):
            for u in range(unroll):
                for prio, lo, sem in ((0, lo0, sem0), (1, lo1, sem1)):
                    sl = pl.ds(pl.multiple_of(lo + (i * unroll + u) * CHUNK_ROWS, CHUNK_ROWS), CHUNK_ROWS)
                    pltpu.make_async_copy(wo_hbm.at[sl], wo_v.at[sl], sem).start(priority=prio)
            return carry

        lax.fori_loop(0, n // (unroll * CHUNK_ROWS), body, 0)

    def start_wo(slab):
        s0, s1 = sems(slab)
        half, n = QW // 2, QW // 4
        if slab == 0:
            start_wo_rows(0, half, n, s0, s1)
        else:
            start_wo_rows(n, half + n, n - WO_TAIL, s0, s1)
            start_wo_rows(2 * n - WO_TAIL, QW - WO_TAIL, WO_TAIL, s0, sem_tail)

    def refill(t, h):
        @pl.when(h + 1 < HKV)
        def _():
            start_kv(t, jnp.minimum(h + 1, HKV - 1))

        @pl.when(h + 1 == HKV)
        def _():
            start_wo(t)

    smalls = [pltpu.make_async_copy(src, dst, sems(0)[0])
              for src, dst in ((x_hbm, x_v), (gw_hbm, gw_v), (b1_hbm, b1_v), (b2_hbm, b2_v))]

    start_wq()
    for c in smalls:
        c.start()
    start_ffn_weights()
    q_scr[...] = jnp.zeros_like(q_scr)
    o_scr[...] = jnp.zeros_like(o_scr)

    s0, s1 = sems(0)
    wait_all(wq_v.at[0:D // 2], s0)
    wait_all(wq_v.at[D // 2:D], s1)
    for c in smalls:
        c.wait()
    x = x_v[...]
    q = jnp.dot(x, wq_v[...], preferred_element_type=f32)
    start_kv(0, 0)
    for hq in range(HQ):
        q_scr[hq // REP, pl.ds(hq % REP, B, stride=8), :] = q[:, hq * DH:(hq + 1) * DH]

    s0, s1 = sems(1)
    wait_all(w1_v, s0)
    hid = jnp.dot(x, w1_v[...], preferred_element_type=f32) + b1_v[...].astype(f32)[None, :]
    hid = jnp.where(hid > 0.0, hid, 0.0)
    hid = (hid * hid).astype(bf16)
    wait_all(w2_v, s1)
    ffn = jnp.dot(hid, w2_v[...], preferred_element_type=f32) + b2_v[...].astype(f32)[None, :]
    g = jax.nn.sigmoid(jnp.sum(x.astype(f32) * gw_v[...].astype(f32)[None, :], axis=-1, keepdims=True))
    mix_scr[...] = (1.0 - g) * ffn
    g_scr[...] = jnp.broadcast_to(g, (B, DH))
    start_kv(1, 0)

    def head_step(h, carry):
        for t in range(B // 2):
            s0, s1 = sems(t)
            wait_all(kbuf.at[2 * t:2 * t + 2], s0)
            wait_all(vbuf.at[2 * t:2 * t + 2], s1)
            outs = []
            for slot in (2 * t, 2 * t + 1):
                b = SLOT_BATCH[slot]
                qb = q_scr[h, b * 8:(b + 1) * 8, :].astype(bf16)
                s = lax.dot_general(qb, kbuf[slot], (((1,), (1,)), ((), ())),
                                    preferred_element_type=f32) * SCALE
                m = jnp.max(s, axis=-1, keepdims=True)
                p = jnp.exp(s - m)
                l = jnp.sum(p, axis=-1, keepdims=True)
                o = jnp.dot(p.astype(bf16), vbuf[slot], preferred_element_type=f32)
                outs.append((b, o, l))
            refill(t, h)
            for b, o, l in outs:
                o_scr[h, pl.ds(b, REP, stride=8), :] = (o / l)[0:REP, :]
        return carry

    lax.fori_loop(0, HKV, head_step, 0)

    (a0, a1), (b0, b1) = sems(0), sems(1)
    half, n = QW // 2, QW // 4
    pieces = [(0, n, a0), (half, half + n, a1), (n, half, b0),
              (half + n, QW - WO_TAIL, b1), (QW - WO_TAIL, QW, sem_tail)]
    acc = None
    for lo, hi, sem in pieces:
        heads = [o_scr[hq // REP, (hq % REP) * 8:(hq % REP + 1) * 8, :] for hq in range(lo // DH, hi // DH)]
        oh = jnp.concatenate(heads, axis=1).astype(bf16)
        wait_all(wo_v.at[lo:hi], sem)
        part = jnp.dot(oh, wo_v[lo:hi, :], preferred_element_type=f32)
        acc = part if acc is None else acc + part
    o_ref[...] = (g_scr[:, 0:1] * acc[0:B, :] + mix_scr[...]).astype(o_ref.dtype)


@jax.jit
def pallas_gated_mix__gqa_block_cached__dense_activation_squared_relu__decode_kernel(
    A_x: jax.Array,
    A_k_cache: jax.Array,
    A_v_cache: jax.Array,
    A_wq: jax.Array,
    A_wo: jax.Array,
    B_x: jax.Array,
    B_w1: jax.Array,
    B_b1: jax.Array,
    B_w2: jax.Array,
    B_b2: jax.Array,
    gate_w: jax.Array,
):
    del B_x
    hbm = pl.BlockSpec(memory_space=pltpu.HBM)
    out = pl.pallas_call(
        _kernel,
        out_shape=jax.ShapeDtypeStruct((B, D), A_x.dtype),
        in_specs=[hbm] * 10,
        out_specs=pl.BlockSpec(memory_space=pltpu.VMEM),
        scratch_shapes=[
            pltpu.VMEM((B, D), bf16),
            pltpu.VMEM((D,), bf16),
            pltpu.VMEM((F,), bf16),
            pltpu.VMEM((D,), bf16),
            pltpu.VMEM((D, QW), bf16),
            pltpu.VMEM((D, F), bf16),
            pltpu.VMEM((F, D), bf16),
            pltpu.VMEM((QW, D), bf16),
            pltpu.VMEM((B, SK, DH), bf16),
            pltpu.VMEM((B, SK, DH), bf16),
            pltpu.VMEM((HKV, B * 8, DH), f32),
            pltpu.VMEM((HKV, REP * 8, DH), f32),
            pltpu.VMEM((B, D), f32),
            pltpu.VMEM((B, DH), f32),
            pltpu.SemaphoreType.DMA((4,)),
            pltpu.SemaphoreType.DMA(()),
        ],
        compiler_params=pltpu.CompilerParams(vmem_limit_bytes=48 * 1024 * 1024),
    )(A_x.reshape(B, D), A_k_cache, A_v_cache, A_wq, A_wo, B_w1, B_b1, B_w2, B_b2, gate_w)
    return out.reshape(B, 1, D)
```

```python
import jax
import jax.numpy as jnp
from jax import lax
import jax.experimental.pallas as pl
import jax.experimental.pallas.tpu as pltpu

B, D, HQ, HKV, SK, DH, F = 4, 512, 32, 8, 4096, 128, 1792
REP = HQ // HKV
QW = HQ * DH
SCALE = float(DH) ** -0.5

CHUNK_ROWS = 16
KV_ROWS = 128
V_LEAD = 5
WO_TAIL = 256
SLOT_BATCH = (0, 2, 1, 3)

f32 = jnp.float32
bf16 = jnp.bfloat16


def _kernel(x_hbm, k_hbm, v_hbm, wq_hbm, wo_hbm, w1_hbm, b1_hbm, w2_hbm, b2_hbm, gw_hbm,
            o_ref,
            x_v, gw_v, b1_v, b2_v, wq_v, w1_v, w2_v, wo_v, kbuf, vbuf,
            q_scr, o_scr, mix_scr, g_scr, sem_ring, sem_tail, sem_small):

    def wait_all(dst, sem):
        pltpu.make_async_copy(dst, dst, sem).wait()

    def sems(i):
        return sem_ring.at[2 * (i % 2)], sem_ring.at[2 * (i % 2) + 1]

    def start_wq():
        s0, s1 = sems(0)

        def body(rg, carry):
            r0 = pl.multiple_of(rg * CHUNK_ROWS, CHUNK_ROWS)
            for c in range(QW // 1024):
                cs = pl.ds(c * 1024, 1024)
                for w in range(2):
                    for prio, sem in ((0, s0), (1, s1)):
                        rs = pl.ds(r0 + prio * (D // 2) + w * (D // 4), CHUNK_ROWS)
                        pltpu.make_async_copy(wq_hbm.at[rs, cs], wq_v.at[rs, cs], sem).start(priority=prio)
            return carry

        lax.fori_loop(0, D // 4 // CHUNK_ROWS, body, 0)

    def start_ffn_weights():
        s0, s1 = sems(1)

        def body(i, carry):
            for a in range(7):
                for w in range(2):
                    if a < 4:
                        sl = pl.ds(pl.multiple_of(w * (D // 2) + (i * 4 + a) * 16, 16), 16)
                        pltpu.make_async_copy(w1_hbm.at[sl], w1_v.at[sl], s0).start(priority=0)
                    sl = pl.ds(pl.multiple_of(w * (F // 2) + (i * 7 + a) * 32, 32), 32)
                    pltpu.make_async_copy(w2_hbm.at[sl], w2_v.at[sl], s1).start(priority=1)
            return carry

        lax.fori_loop(0, 4, body, 0)

    def start_kv(t, h):
        s0, s1 = sems(t)
        unroll, nchunk = 4, SK // KV_ROWS

        def body(i, carry):
            for u in range(unroll):
                j = i * unroll + u
                ksl = pl.ds(pl.multiple_of(j * KV_ROWS, KV_ROWS), KV_ROWS)
                vsl = pl.ds(pl.multiple_of(lax.rem(j + V_LEAD, nchunk) * KV_ROWS, KV_ROWS), KV_ROWS)
                for slot in (2 * t, 2 * t + 1):
                    b = SLOT_BATCH[slot]
                    pltpu.make_async_copy(k_hbm.at[b, h, ksl], kbuf.at[slot, ksl], s0).start(priority=0)
                    pltpu.make_async_copy(v_hbm.at[b, h, vsl], vbuf.at[slot, vsl], s1).start(priority=1)
            return carry

        lax.fori_loop(0, nchunk // unroll, body, 0)

    def start_wo_rows(lo0, lo1, n, sem0, sem1):
        unroll = 8
        assert n % (unroll * CHUNK_ROWS) == 0

        def body(i, carry):
            for u in range(unroll):
                for prio, lo, sem in ((0, lo0, sem0), (1, lo1, sem1)):
                    sl = pl.ds(pl.multiple_of(lo + (i * unroll + u) * CHUNK_ROWS, CHUNK_ROWS), CHUNK_ROWS)
                    pltpu.make_async_copy(wo_hbm.at[sl], wo_v.at[sl], sem).start(priority=prio)
            return carry

        lax.fori_loop(0, n // (unroll * CHUNK_ROWS), body, 0)

    def start_wo(slab):
        s0, s1 = sems(slab)
        half, n = QW // 2, QW // 4
        if slab == 0:
            start_wo_rows(0, half, n, s0, s1)
        else:
            start_wo_rows(n, half + n, n - WO_TAIL, s0, s1)
            start_wo_rows(2 * n - WO_TAIL, QW - WO_TAIL, WO_TAIL, s0, sem_tail)

    def refill(t, h):
        @pl.when(h + 1 < HKV)
        def _():
            start_kv(t, jnp.minimum(h + 1, HKV - 1))

        @pl.when(h + 1 == HKV)
        def _():
            start_wo(t)

    smalls = [pltpu.make_async_copy(src, dst, sem_small)
              for src, dst in ((x_hbm, x_v), (gw_hbm, gw_v), (b1_hbm, b1_v), (b2_hbm, b2_v))]

    start_wq()
    for c in smalls:
        c.start()
    start_ffn_weights()
    q_scr[...] = jnp.zeros_like(q_scr)
    o_scr[...] = jnp.zeros_like(o_scr)

    s0, s1 = sems(0)
    wait_all(wq_v.at[0:D // 2], s0)
    wait_all(wq_v.at[D // 2:D], s1)
    for c in smalls:
        c.wait()
    x = x_v[...]
    q = jnp.dot(x, wq_v[...], preferred_element_type=f32)
    start_kv(0, 0)
    for hq in range(HQ):
        q_scr[hq // REP, pl.ds(hq % REP, B, stride=8), :] = q[:, hq * DH:(hq + 1) * DH]

    s0, s1 = sems(1)
    wait_all(w1_v, s0)
    hid = jnp.dot(x, w1_v[...], preferred_element_type=f32) + b1_v[...].astype(f32)[None, :]
    hid = jnp.where(hid > 0.0, hid, 0.0)
    hid = (hid * hid).astype(bf16)
    wait_all(w2_v, s1)
    ffn = jnp.dot(hid, w2_v[...], preferred_element_type=f32) + b2_v[...].astype(f32)[None, :]
    g = jax.nn.sigmoid(jnp.sum(x.astype(f32) * gw_v[...].astype(f32)[None, :], axis=-1, keepdims=True))
    mix_scr[...] = (1.0 - g) * ffn
    g_scr[...] = jnp.broadcast_to(g, (B, DH))
    start_kv(1, 0)

    def head_step(h, carry):
        for t in range(B // 2):
            s0, s1 = sems(t)
            wait_all(kbuf.at[2 * t:2 * t + 2], s0)
            wait_all(vbuf.at[2 * t:2 * t + 2], s1)
            outs = []
            for slot in (2 * t, 2 * t + 1):
                b = SLOT_BATCH[slot]
                qb = q_scr[h, b * 8:(b + 1) * 8, :].astype(bf16)
                s = lax.dot_general(qb, kbuf[slot], (((1,), (1,)), ((), ())),
                                    preferred_element_type=f32) * SCALE
                m = jnp.max(s, axis=-1, keepdims=True)
                p = jnp.exp(s - m)
                l = jnp.sum(p, axis=-1, keepdims=True)
                o = jnp.dot(p.astype(bf16), vbuf[slot], preferred_element_type=f32)
                outs.append((b, o, l))
            refill(t, h)
            for b, o, l in outs:
                o_scr[h, pl.ds(b, REP, stride=8), :] = (o / l)[0:REP, :]
        return carry

    lax.fori_loop(0, HKV, head_step, 0)

    (a0, a1), (b0, b1) = sems(0), sems(1)
    half, n = QW // 2, QW // 4
    pieces = [(0, n, a0), (half, half + n, a1), (n, half, b0),
              (half + n, QW - WO_TAIL, b1), (QW - WO_TAIL, QW, sem_tail)]
    acc = None
    for lo, hi, sem in pieces:
        heads = [o_scr[hq // REP, (hq % REP) * 8:(hq % REP + 1) * 8, :] for hq in range(lo // DH, hi // DH)]
        oh = jnp.concatenate(heads, axis=1).astype(bf16)
        wait_all(wo_v.at[lo:hi], sem)
        part = jnp.dot(oh, wo_v[lo:hi, :], preferred_element_type=f32)
        acc = part if acc is None else acc + part
    o_ref[...] = (g_scr[:, 0:1] * acc[0:B, :] + mix_scr[...]).astype(o_ref.dtype)


@jax.jit
def pallas_gated_mix__gqa_block_cached__dense_activation_squared_relu__decode_kernel(
    A_x: jax.Array,
    A_k_cache: jax.Array,
    A_v_cache: jax.Array,
    A_wq: jax.Array,
    A_wo: jax.Array,
    B_x: jax.Array,
    B_w1: jax.Array,
    B_b1: jax.Array,
    B_w2: jax.Array,
    B_b2: jax.Array,
    gate_w: jax.Array,
):
    del B_x
    hbm = pl.BlockSpec(memory_space=pltpu.HBM)
    out = pl.pallas_call(
        _kernel,
        out_shape=jax.ShapeDtypeStruct((B, D), A_x.dtype),
        in_specs=[hbm] * 10,
        out_specs=pl.BlockSpec(memory_space=pltpu.VMEM),
        scratch_shapes=[
            pltpu.VMEM((B, D), bf16),
            pltpu.VMEM((D,), bf16),
            pltpu.VMEM((F,), bf16),
            pltpu.VMEM((D,), bf16),
            pltpu.VMEM((D, QW), bf16),
            pltpu.VMEM((D, F), bf16),
            pltpu.VMEM((F, D), bf16),
            pltpu.VMEM((QW, D), bf16),
            pltpu.VMEM((B, SK, DH), bf16),
            pltpu.VMEM((B, SK, DH), bf16),
            pltpu.VMEM((HKV, B * 8, DH), f32),
            pltpu.VMEM((HKV, REP * 8, DH), f32),
            pltpu.VMEM((B, D), f32),
            pltpu.VMEM((B, DH), f32),
            pltpu.SemaphoreType.DMA((4,)),
            pltpu.SemaphoreType.DMA(()),
            pltpu.SemaphoreType.DMA(()),
        ],
        compiler_params=pltpu.CompilerParams(vmem_limit_bytes=48 * 1024 * 1024),
    )(A_x.reshape(B, D), A_k_cache, A_v_cache, A_wq, A_wo, B_w1, B_b1, B_w2, B_b2, gate_w)
    return out.reshape(B, 1, D)
```
